```python
import os as _os
_os.environ.setdefault("JAX_PLATFORMS", "cpu")
import jax
import jax.numpy as jnp

def _softmax(x, axis=-1):
    return jax.nn.softmax(x, axis=axis)
def _gelu(x):
    return jax.nn.gelu(x, approximate=True)
def _silu(x):
    return jax.nn.silu(x)
def _sigmoid(x):
    return jax.nn.sigmoid(x)
def _layernorm(x, axis=-1, eps=1e-5):
    m = jnp.mean(x, axis=axis, keepdims=True)
    v = jnp.var(x, axis=axis, keepdims=True)
    return (x - m) / jnp.sqrt(v + eps)
def _scatter_add(tgt, idx, src, axis=0):
    return tgt.at[idx].add(src)
def _segment_sum(src, seg, n):
    return jax.ops.segment_sum(src, seg, n)
class _Rng:
    def __init__(self, key):
        self._k = key
    def _next(self):
        self._k, sub = jax.random.split(self._k)
        return sub
    def normal(self, shape):
        return jax.random.normal(self._next(), shape, dtype=jnp.bfloat16)
    def randint(self, lo, hi, shape):
        return jax.random.randint(self._next(), shape, lo, hi, dtype=jnp.int32)
    def uniform(self, shape, lo=0.0, hi=1.0):
        return jax.random.uniform(self._next(), shape, jnp.bfloat16, lo, hi)
    def permutation(self, n):
        return jax.random.permutation(self._next(), n)


kernel_name = 'sequential_preLN__softmax_full_mha__mixer_channel_mlp__prompt'

def setup_inputs():
    _rng = _Rng(jax.random.key(int.from_bytes(__import__("os").urandom(4), "little")))
    _w = (lambda a: (lambda t: t.astype(jnp.bfloat16) if jnp.issubdtype(t.dtype, jnp.floating) else t)(jnp.asarray(a)))
    def _A_setup():
        B, S, D = 1, 2048, 1024
        return {
            "x": _w((lambda *s: _rng.normal(s) * 0.05)(B, S, D)),
            "wqkv": _w((lambda *s: _rng.normal(s) * 0.05)(D, 3 * D)),
            "wo": _w((lambda *s: _rng.normal(s) * 0.05)(D, D)),
        }
    _A_in = _A_setup()

    def _B_setup():
        B, S, D, F = 1, 2048, 1024, 3584
        return {
            "x": _w((lambda *s: _rng.normal(s) * 0.05)(B, S, D)),
            "w1": _w((lambda *s: _rng.normal(s) * 0.8)(D, F) * (D ** -0.5)),
            "b1": _w((lambda *s: _rng.normal(s) * 0.8)(F)),
            "w2": _w((lambda *s: _rng.normal(s) * 0.8)(F, D) * (F ** -0.5)),
            "b2": _w((lambda *s: _rng.normal(s) * 0.05)(D)),
        }
    _B_in = _B_setup()

    return {
        "A_x": _A_in["x"],
        "A_wqkv": _A_in["wqkv"],
        "A_wo": _A_in["wo"],
        "B_x": _B_in["x"],
        "B_w1": _B_in["w1"],
        "B_b1": _B_in["b1"],
        "B_w2": _B_in["w2"],
        "B_b2": _B_in["b2"],
    }

def reference(A_x, A_wqkv, A_wo, B_x, B_w1, B_b1, B_w2, B_b2):
    def _A_ref(x, wqkv, wo):
        B, S, D = x.shape
        H = 32; Dh = D // H
        qkv = (lambda x, *d: x.transpose(*d))((x @ wqkv).reshape(B, S, 3, H, Dh), 2, 0, 3, 1, 4)
        q, k, v = qkv[0], qkv[1], qkv[2]
        scale = Dh ** -0.5
        scores = jnp.einsum("bhqd,bhkd->bhqk", q, k) * scale
        p = _softmax(scores, axis=-1)
        o = jnp.einsum("bhqk,bhkd->bhqd", p, v)
        return (lambda x, *d: x.transpose(*d))(o, 0, 2, 1, 3).reshape(B, S, D) @ wo

    def _B_ref(x, w1, b1, w2, b2):
        y = _layernorm(x, axis=-1)
        h = _gelu(jnp.einsum("bsd,df->bsf", y, w1) + b1)
        return jnp.einsum("bsf,fd->bsd", h, w2) + b2

    x = A_x
    h = x + _A_ref(_layernorm(x, axis=-1), A_wqkv, A_wo)
    h2 = h + _B_ref(_layernorm(h, axis=-1), B_w1, B_b1, B_w2, B_b2)
    return h2
```

```python
import functools
import numpy as np
import jax
import jax.numpy as jnp
from jax import lax
from jax.experimental import pallas as pl
from jax.experimental.pallas import tpu as pltpu

f32, bf16, u32 = jnp.float32, jnp.bfloat16, jnp.uint32
H = 32
EPS = 1e-5
LOG2E = 1.4426950408889634


def _tree(op, x):
    parts = [x[i * 8:(i + 1) * 8] for i in range(x.shape[0] // 8)]
    while len(parts) > 1:
        nxt = [op(parts[i], parts[i + 1]) for i in range(0, len(parts) - 1, 2)]
        if len(parts) % 2:
            nxt.append(parts[-1])
        parts = nxt
    return parts[0]


def _ln(x):
    mu = jnp.mean(x, axis=-1, keepdims=True)
    xc = x - mu
    var = jnp.mean(xc * xc, axis=-1, keepdims=True)
    return xc * lax.rsqrt(var + EPS)


def _gelu(x):
    c = 0.7978845608028654
    u = x * (c + (c * 0.044715) * (x * x))
    hx = 0.5 * x
    return hx + hx * jnp.tanh(u)


def _pack(x):
    return pltpu.bitcast(x.astype(bf16), u32)


def _unpack(x):
    return pltpu.bitcast(x, bf16)


def make(S, D, F, bm1=256, bq=512, kc=128, bm3=256, fc=512):
    Dh = D // H
    G = D // 128
    HPS = 128 // Dh
    nq = S // bq
    nb1 = S // bm1
    nb3 = S // bm3
    qscale = (Dh ** -0.5) * LOG2E

    def kernel(x_hbm, wqkv_hbm, wo_hbm, w1_hbm, b1_hbm, w2_hbm, b2_hbm, out_hbm,
               x_v, wqkv_v, wo_v, w1_v, b1_v, w2_v, b2_v,
               y_s, k_s, qt_s, vt_s, s_buf, out_v, sem_x, sem_w, sem_o):
        def x_copy(i):
            return pltpu.make_async_copy(x_hbm.at[pl.ds(i * bm1, bm1)], x_v.at[pl.ds(i * bm1, bm1)], sem_x.at[i])
        w_copies = [
            pltpu.make_async_copy(wqkv_hbm, wqkv_v, sem_w.at[0]),
            pltpu.make_async_copy(wo_hbm, wo_v, sem_w.at[1]),
            pltpu.make_async_copy(w1_hbm, w1_v, sem_w.at[2]),
            pltpu.make_async_copy(w2_hbm, w2_v, sem_w.at[3]),
            pltpu.make_async_copy(b1_hbm, b1_v, sem_w.at[4]),
            pltpu.make_async_copy(b2_hbm, b2_v, sem_w.at[5]),
        ]
        x_copy(0).start()
        w_copies[0].start()
        for i in range(1, nb1):
            x_copy(i).start()
        for c in w_copies[1:]:
            c.start()

        def ln_block(i):
            r = pl.multiple_of(i * bm1, bm1)
            rh = pl.multiple_of(i * (bm1 // 2), bm1 // 2)
            y_s[pl.ds(rh, bm1 // 2), :] = _pack(_ln(x_v[pl.ds(r, bm1), :].astype(f32)))

        x_copy(0).wait()
        ln_block(0)
        for i in range(1, nb1):
            x_copy(i).wait()
        w_copies[0].wait()

        def p1(i, c):
            r = pl.multiple_of(i * bm1, bm1)
            rh = pl.multiple_of(i * (bm1 // 2), bm1 // 2)
            y = _unpack(y_s[pl.ds(rh, bm1 // 2), :])
            q = jnp.dot(y, wqkv_v[:, 0:D], preferred_element_type=f32) * qscale
            qt_s[:, pl.ds(r, bm1)] = _pack(q.T)
            k = jnp.dot(y, wqkv_v[:, D:2 * D], preferred_element_type=f32)
            k_s[pl.ds(rh, bm1 // 2), :] = _pack(k)
            v = jnp.dot(y, wqkv_v[:, 2 * D:3 * D], preferred_element_type=f32)
            vt_s[:, pl.ds(r, bm1)] = _pack(v.T)
            ln_block(jnp.minimum(i + 1, nb1 - 1))
            return c
        lax.fori_loop(0, nb1, p1, 0)

        hr = Dh // 2

        def masked_q(it, j):
            qb = it // G
            g = it % G
            q0 = pl.multiple_of(qb * bq, bq)
            r0 = pl.multiple_of(g * 64 + j * hr, hr)
            qh = qt_s[pl.ds(r0, hr), pl.ds(q0, bq)]
            parts = []
            if j > 0:
                parts.append(jnp.zeros((j * hr, bq), u32))
            parts.append(qh)
            if j < HPS - 1:
                parts.append(jnp.zeros(((HPS - 1 - j) * hr, bq), u32))
            return _unpack(jnp.concatenate(parts, axis=0))

        def stage(it_a, j_a, it_b, j_b, src, m):
            do_a, do_b = it_a is not None, it_b is not None
            if do_a:
                qm = masked_q(it_a, j_a)
                ga = pl.multiple_of((it_a % G) * 128, 128)
            if do_b:
                rb = pl.multiple_of((it_b % G) * 64 + j_b * hr, hr)
            mx = l = o = None
            outs = []
            for ci, c0 in enumerate(range(0, S, kc)):
                if do_b:
                    p = jnp.exp2(src(ci) - m)
                    lc = _tree(jnp.add, p)
                    vv = _unpack(vt_s[pl.ds(rb, hr), c0:c0 + kc])
                    oc = jnp.dot(vv, p.astype(bf16), preferred_element_type=f32)
                    l = lc if l is None else l + lc
                    o = oc if o is None else o + oc
                if do_a:
                    kk = _unpack(k_s[c0 // 2:(c0 + kc) // 2, pl.ds(ga, 128)])
                    s = jnp.dot(kk, qm, preferred_element_type=f32)
                    outs.append(s)
                    mc = _tree(jnp.maximum, s)
                    mx = mc if mx is None else jnp.maximum(mx, mc)
            on = mn = None
            if do_b:
                on = o * (1.0 / jnp.sum(l, axis=0, keepdims=True))
            if do_a:
                mn = jnp.max(mx, axis=0, keepdims=True)
            return outs, mn, on

        def store_s(outs):
            for ci, s in enumerate(outs):
                s_buf[ci * kc:(ci + 1) * kc, :] = s

        n_it = nq * G
        outs, m0, _ = stage(0, 0, None, None, None, None)
        store_s(outs)

        def p2(it, m):
            src = lambda ci: s_buf[ci * kc:(ci + 1) * kc, :]
            os_ = []
            for j in range(HPS):
                if j < HPS - 1:
                    outs, m, on = stage(it, j + 1, it, j, src, m)
                    src = (lambda outs: (lambda ci: outs[ci]))(outs)
                else:
                    outs, m, on = stage(jnp.minimum(it + 1, n_it - 1), 0, it, j, src, m)
                    store_s(outs)
                os_.append(on)
            ot = jnp.concatenate(os_, axis=0)
            qh = pl.multiple_of((it // G) * (bq // 2), bq // 2)
            g0 = pl.multiple_of((it % G) * 128, 128)
            y_s[pl.ds(qh, bq // 2), pl.ds(g0, 128)] = _pack(ot.T)
            return m
        lax.fori_loop(0, n_it, p2, m0)

        for c in w_copies[1:]:
            c.wait()

        def o_copy(i, slot):
            return pltpu.make_async_copy(out_v.at[slot], out_hbm.at[pl.ds(i * bm3, bm3)], sem_o.at[slot])

        def p3(i, c):
            slot = i % 2
            r = pl.multiple_of(i * bm3, bm3)
            rh = pl.multiple_of(i * (bm3 // 2), bm3 // 2)

            @pl.when(i >= 2)
            def _():
                o_copy(i - 2, slot).wait()
            o = _unpack(y_s[pl.ds(rh, bm3 // 2), :])
            h = x_v[pl.ds(r, bm3), :].astype(f32) + jnp.dot(o, wo_v[...], preferred_element_type=f32)
            y2 = _ln(h).astype(bf16)
            acc = h + b2_v[...].astype(f32)
            for f0 in range(0, F, fc):
                a = jnp.dot(y2, w1_v[:, f0:f0 + fc], preferred_element_type=f32) + b1_v[:, f0:f0 + fc].astype(f32)
                acc = acc + jnp.dot(_gelu(a).astype(bf16), w2_v[f0:f0 + fc, :], preferred_element_type=f32)
            out_v[slot] = acc.astype(bf16)
            o_copy(i, slot).start()
            return c
        lax.fori_loop(0, nb3, p3, 0)
        o_copy(nb3 - 2, (nb3 - 2) % 2).wait()
        o_copy(nb3 - 1, (nb3 - 1) % 2).wait()

    any_spec = pl.BlockSpec(memory_space=pl.ANY)
    return pl.pallas_call(
        kernel,
        out_shape=jax.ShapeDtypeStruct((S, D), bf16),
        in_specs=[any_spec] * 7,
        out_specs=any_spec,
        scratch_shapes=[
            pltpu.VMEM((S, D), bf16), pltpu.VMEM((D, 3 * D), bf16), pltpu.VMEM((D, D), bf16),
            pltpu.VMEM((D, F), bf16), pltpu.VMEM((1, F), bf16), pltpu.VMEM((F, D), bf16), pltpu.VMEM((1, D), bf16),
            pltpu.VMEM((S // 2, D), u32), pltpu.VMEM((S // 2, D), u32),
            pltpu.VMEM((D // 2, S), u32), pltpu.VMEM((D // 2, S), u32),
            pltpu.VMEM((S, bq), f32), pltpu.VMEM((2, bm3, D), bf16),
            pltpu.SemaphoreType.DMA((nb1,)), pltpu.SemaphoreType.DMA((6,)), pltpu.SemaphoreType.DMA((2,)),
        ],
        compiler_params=pltpu.CompilerParams(vmem_limit_bytes=110 * 2**20),
        name="fused_block",
    )


@jax.jit
def pallas_sequential_preLN__softmax_full_mha__mixer_channel_mlp__prompt_kernel(
    A_x, A_wqkv, A_wo, B_x, B_w1, B_b1, B_w2, B_b2):
    del B_x
    B, S, D = A_x.shape
    F = B_w1.shape[1]
    out = make(S, D, F)(A_x.reshape(S, D), A_wqkv, A_wo, B_w1, B_b1.reshape(1, F), B_w2, B_b2.reshape(1, D))
    return out.reshape(B, S, D)
```

```python
import numpy as np
import jax
import jax.numpy as jnp
from jax import lax
from jax.experimental import pallas as pl
from jax.experimental.pallas import tpu as pltpu

f32, bf16, u32 = jnp.float32, jnp.bfloat16, jnp.uint32
H = 32
EPS = 1e-5
LOG2E = 1.4426950408889634


def _tree(op, x):
    parts = [x[i * 8:(i + 1) * 8] for i in range(x.shape[0] // 8)]
    while len(parts) > 1:
        nxt = [op(parts[i], parts[i + 1]) for i in range(0, len(parts) - 1, 2)]
        if len(parts) % 2:
            nxt.append(parts[-1])
        parts = nxt
    return parts[0]


def _ln(x, keep_centered=True):
    mu = jnp.mean(x, axis=-1, keepdims=True)
    xc = x - mu
    r = lax.rsqrt(jnp.mean(xc * xc, axis=-1, keepdims=True) + EPS)
    return xc * r if keep_centered else x * r - mu * r


def _gelu(x):
    c = 0.7978845608028654
    u = x * (c + (c * 0.044715) * (x * x))
    hx = 0.5 * x
    return hx + hx * jnp.tanh(u)


def _pack(x):
    return pltpu.bitcast(x.astype(bf16), u32)


def _unpack(x):
    return pltpu.bitcast(x, bf16)


def _dot(a, b):
    return jnp.dot(a, b, preferred_element_type=f32)


def _grid(x, n):
    r, c = x.shape[0] // n, x.shape[1] // n
    return [[x[i * r:(i + 1) * r, j * c:(j + 1) * c] for j in range(n)] for i in range(n)]


def _add(a, b):
    return [[u + v for u, v in zip(ra, rb)] for ra, rb in zip(a, b)]


def _sub(a, b):
    return [[u - v for u, v in zip(ra, rb)] for ra, rb in zip(a, b)]


def _quads(g):
    h = len(g) // 2
    return ([r[:h] for r in g[:h]], [r[h:] for r in g[:h]], [r[:h] for r in g[h:]], [r[h:] for r in g[h:]])


def _lhs_ops(g):
    if len(g) == 1:
        return [g[0][0]]
    a11, a12, a21, a22 = _quads(g)
    ops = (_add(a11, a22), _add(a21, a22), a11, a22, _add(a11, a12), _sub(a21, a11), _sub(a12, a22))
    return [v for q in ops for v in _lhs_ops(q)]


def _rhs_ops(g):
    if len(g) == 1:
        return [g[0][0]]
    b11, b12, b21, b22 = _quads(g)
    ops = (_add(b11, b22), b11, _sub(b12, b22), _sub(b21, b11), b22, _add(b11, b12), _add(b21, b22))
    return [v for q in ops for v in _rhs_ops(q)]


def _strassen(prod, lvl, base=0):
    if lvl == 0:
        return [[prod(base)]]
    m = lambda i: _strassen(prod, lvl - 1, base + i * 7 ** (lvl - 1))
    m3 = m(2)
    m5 = m(4)
    c12 = _add(m3, m5)
    m1 = m(0)
    c22 = _add(m1, m3)
    c11 = _sub(m1, m5)
    m4 = m(3)
    c11 = _add(_add(c11, m4), m(6))
    m2 = m(1)
    c21 = _add(m2, m4)
    c22 = _add(_sub(c22, m2), m(5))
    return [l + r for l, r in zip(c11, c12)] + [l + r for l, r in zip(c21, c22)]


def make(S, D, F, bm1=256, bq=256, kc=128, lag=3, U=4, bm3=256, lq=1, lo=2, lm=2, n_early=2, nsub=128, psub=128, prow=128, split=(0.3, 0.9), jlo=8, jhi=16):
    Dh = D // H
    G = D // 128
    HPS = 128 // Dh
    nq = S // bq
    nb1 = S // bm1
    nb3 = S // bm3
    qscale = (Dh ** -0.5) * LOG2E
    WC = 512
    nwc = 3 * D // WC
    gq, go, gm = 2 ** lq, 2 ** lo, 2 ** lm
    NP = nb1 - 1
    fw = F // gm // NP
    PAD = 16

    def kernel(x_hbm, wqkv_hbm, wo_hbm, w1_hbm, b1_hbm, w2_hbm, b2_hbm, out_hbm,
               x_v, wq0, wq1, wq2, wq3, wq4, wq5, wo_v, w1_v, b1_v, w2_v, b2_v,
               wqkv_c, wo_c, w1_c, w2_c, l_s, g_s,
               o_s, k_s, qt_s, vt_s, sb0, sb1, sb2, sb3, ot_s, st_mx, st_m, st_l, st_o, out_v,
               sem_x, sem_q, sem_w, sem_p, sem_o):
        sb = [sb0, sb1, sb2, sb3]
        wq_v = [wq0, wq1, wq2, wq3, wq4, wq5]

        def x_copy(i):
            return pltpu.make_async_copy(x_hbm.at[pl.ds(i * bm1, bm1)], x_v.at[pl.ds(i * bm1, bm1)], sem_x.at[i])

        def q_copy(n):
            return pltpu.make_async_copy(wqkv_hbm.at[:, pl.ds(n * WC, WC)], wq_v[n].at[pl.ds(0, D)], sem_q.at[n])

        w_copies = [
            pltpu.make_async_copy(wo_hbm, wo_v.at[pl.ds(0, D)], sem_w.at[0]),
            pltpu.make_async_copy(b1_hbm, b1_v, sem_w.at[1]),
            pltpu.make_async_copy(b2_hbm, b2_v, sem_w.at[2]),
        ]

        def piece_copies(p, slot):
            pw = gm * fw
            f0 = p * pw if isinstance(p, int) else pl.multiple_of(p * pw, pw)
            return [pltpu.make_async_copy(w1_hbm.at[:, pl.ds(f0, pw)], w1_v.at[pl.ds(slot * D, D)], sem_p.at[2 * slot]),
                    pltpu.make_async_copy(w2_hbm.at[pl.ds(f0, pw)], w2_v.at[pl.ds(slot * pw, pw)], sem_p.at[2 * slot + 1])]

        def fence(raw, col, val, z):
            top = raw.shape[0] - PAD
            row = pl.multiple_of(jnp.clip(z + top, 0, top), PAD)
            raw[pl.ds(row, PAD), col:col + 128] = val[0:PAD, 0:128].astype(bf16)

        def combine(load, n, store, outer=None):
            if outer is None:
                for idx, v in enumerate(_rhs_ops([[load(i, j).astype(f32) for j in range(n)] for i in range(n)])):
                    store(idx, _pack(v))
                return
            h = n // 2
            quad = lambda a, b: [[load(a * h + i, b * h + j).astype(f32) for j in range(h)] for i in range(h)]
            op, a, b = ((_add, (0, 0), (1, 1)), (None, (0, 0), None), (_sub, (0, 1), (1, 1)), (_sub, (1, 0), (0, 0)),
                        (None, (1, 1), None), (_add, (0, 0), (0, 1)), (_add, (1, 0), (1, 1)))[outer]
            ops = _rhs_ops(quad(*a) if op is None else op(quad(*a), quad(*b)))
            for idx, v in enumerate(ops):
                store(outer * len(ops) + idx, _pack(v))

        def put_qkv(which, t0, c0, val):
            n, w = val.shape
            if which == 0:
                qt_s[c0 // 2:(c0 + w) // 2, pl.ds(t0, n)] = _pack((val * qscale).T)
            elif which == 2:
                vt_s[c0 // 2:(c0 + w) // 2, pl.ds(t0, n)] = _pack(val.T)
            else:
                th = t0 // 2 if isinstance(t0, int) else pl.multiple_of(t0 // 2, n // 2)
                k_s[pl.ds(th, n // 2), c0:c0 + w] = _pack(val)

        tq = bm1 // gq
        kq = D // gq

        def ln_operands(i):
            r = i * bm1 if isinstance(i, int) else pl.multiple_of(i * bm1, bm1)
            for j, v in enumerate(_lhs_ops(_grid(_ln(x_v[pl.ds(r, bm1), :].astype(f32)), gq))):
                l_s[j * (tq // 2):(j + 1) * (tq // 2), :] = _pack(v)

        km, fm = D // gm, F // gm

        def mlp_jobs(p, slot):
            jobs = []
            static = isinstance(p, int)
            mo = lambda v, k: v if isinstance(v, int) else pl.multiple_of(v, k)
            n1 = p * fw
            outers = range(7) if lm > 1 else [None]
            first_col = lambda o: gm // 2 if o in (2, 4) else 0
            for r0 in range(0, km, 16):
                for c0 in range(0, fw, 128):
                    load = lambda a, b, r0=r0, c0=c0: w1_v[pl.ds(mo(slot * D + a * km + r0, 16), 16), b * fw + c0:b * fw + c0 + 128]

                    def store(idx, v, r0=r0, c0=c0):
                        w1_c[idx * (km // 2) + r0 // 2:idx * (km // 2) + r0 // 2 + 8, pl.ds(mo(n1 + c0, 128), 128)] = v
                    jobs.extend((w1_v, first_col(o) * fw + c0, load, gm, store, o) for o in outers)
            for r0 in range(0, fw, 16):
                for c0 in range(0, km, 128):
                    load = lambda a, b, r0=r0, c0=c0: w2_v[pl.ds(mo((slot * gm + a) * fw + r0, 16), 16), b * km + c0:b * km + c0 + 128]

                    def store(idx, v, r0=r0, c0=c0):
                        w2_c[pl.ds(mo(idx * (fm // 2) + (n1 + r0) // 2, 8), 8), c0:c0 + 128] = v
                    jobs.extend((w2_v, first_col(o) * km + c0, load, gm, store, o) for o in outers)
            return jobs

        def qkv_jobs(which):
            jobs = []
            for r0 in range(0, kq, 16):
                for n0 in range(0, kq, 128):
                    load = lambda a, b, r0=r0, n0=n0: wq_v[2 * which + b][a * kq + r0:a * kq + r0 + 16, n0:n0 + 128]

                    def store(idx, v, r0=r0, n0=n0):
                        r = (which * 7 ** lq + idx) * (kq // 2) + r0 // 2
                        wqkv_c[r:r + 8, n0:n0 + 128] = v
                    jobs.append((wq_v[2 * which], n0, load, gq, store, None))
            return jobs

        def run_jobs(jobs, n, nslots, val, z):
            for raw, col, load, g, store, outer in jobs[n * len(jobs) // nslots:(n + 1) * len(jobs) // nslots]:
                fence(raw, col, val, z)
                combine(load, g, store, outer)

        def opaque_zero():
            v = pltpu.bitcast(x_v[0:16, 0:128], jnp.int32)[0, 0]
            z = (v * v + v) & 1
            w = pltpu.bitcast(x_v[pl.ds(pl.multiple_of(z * 16, 16), 16), 0:128], jnp.int32)[0, 0]
            return v - w

        def plain(y, t0, chunks, jobs, z):
            nslots = len(chunks) * (WC // psub) * (y.shape[0] // prow) - 2
            n = 0
            for ch in chunks:
                for c in range(ch * WC, (ch + 1) * WC, psub):
                    w = wq_v[ch][0:D, c - ch * WC:c - ch * WC + psub]
                    for r in range(0, y.shape[0], prow):
                        v = _dot(y[r:r + prow], w)
                        put_qkv(c // D, t0 + r, c % D, v)
                        if n < nslots:
                            run_jobs(jobs, n, nslots, v, z)
                        n += 1

        x_copy(0).start()
        q_copy(0).start()
        x_copy(0).wait()
        x_copy(1).start()
        y0 = _ln(x_v[0:bm1, :].astype(f32)).astype(bf16)
        z = opaque_zero()
        q_copy(0).wait()
        q_copy(1).start()
        q_copy(4).start()
        x_copy(1).wait()
        for c in [q_copy(5)] + piece_copies(0, 0):
            c.start()
        plain(y0, 0, [0], [], 0)
        y1 = _ln(x_v[bm1:2 * bm1, :].astype(f32)).astype(bf16)
        plain(y1, bm1, [0], [], 0)
        y01 = jnp.concatenate([y0, y1], axis=0)
        q_copy(1).wait()
        q_copy(4).wait()
        for c in (q_copy(2), q_copy(3), x_copy(2)):
            c.start()
        plain(y01, 0, [1, 4], qkv_jobs(0), z)
        for c in [q_copy(5)] + piece_copies(0, 0):
            c.wait()
        for c in piece_copies(1, 1) + [x_copy(3)]:
            c.start()
        jobs = mlp_jobs(0, 0)
        j1, j2 = int(len(jobs) * split[0]), int(len(jobs) * split[1])
        plain(y01, 0, [5], qkv_jobs(2) + jobs[:j1], z)
        q_copy(2).wait()
        q_copy(3).wait()
        x_copy(2).wait()
        plain(y01, 0, [2], jobs[j1:j2], z)
        plain(y01, 0, [3], jobs[j2:] + qkv_jobs(1), z)
        ln_operands(2)

        def p1(i, carry):
            slot = (i - 1) % 2
            for c in piece_copies(i - 1, slot):
                c.wait()

            @pl.when(i + 1 < nb1)
            def _():
                x_copy(i + 1).wait()
                for c in piece_copies(i, 1 - slot):
                    c.start()

            @pl.when(i + 2 < nb1)
            def _():
                x_copy(i + 2).start()

            @pl.when(i == nb1 - 2)
            def _():
                for c in w_copies:
                    c.start()

            jobs = mlp_jobs(i - 1, slot)
            slots = [n for n in range(jlo, 3 * 7 ** lq * (kq // nsub) - jhi)]
            count = [0]
            z = jnp.minimum(i, 0)

            for which in (0, 2, 1):
                def prod(j):
                    r = (which * 7 ** lq + j) * (kq // 2)
                    lhs = _unpack(l_s[j * (tq // 2):(j + 1) * (tq // 2), :])
                    cols = []
                    for c in range(0, kq, nsub):
                        cols.append(_dot(lhs, _unpack(wqkv_c[r:r + kq // 2, c:c + nsub])))
                        if count[0] in slots:
                            run_jobs(jobs, slots.index(count[0]), len(slots), cols[-1], z)
                        count[0] += 1
                    return jnp.concatenate(cols, axis=1)
                for a, row in enumerate(_strassen(prod, lq)):
                    for b, blk in enumerate(row):
                        put_qkv(which, pl.multiple_of(i * bm1 + a * tq, tq), b * kq, blk)
            ln_operands(jnp.minimum(i + 1, nb1 - 1))
            return carry
        lax.fori_loop(2, nb1, p1, 0)

        hr = Dh // 2
        NC = S // kc
        UN = U * HPS
        npg = G // U
        n_it = nq * npg

        def slab(it, u):
            return u // HPS if npg == 1 else (it % npg) * U + u // HPS

        def off(v, mult):
            return v * mult if isinstance(v, int) else pl.multiple_of(v * mult, mult)

        def masked_q(it, u):
            j = u % HPS
            r0 = slab(it, u) * 64 + j * hr
            if not isinstance(r0, int):
                r0 = pl.multiple_of(r0, hr)
            qh = qt_s[pl.ds(r0, hr), pl.ds(off(it // npg, bq), bq)]
            parts = []
            if j > 0:
                parts.append(jnp.zeros((j * hr, bq), u32))
            parts.append(qh)
            if j < HPS - 1:
                parts.append(jnp.zeros(((HPS - 1 - j) * hr, bq), u32))
            return _unpack(jnp.concatenate(parts, axis=0))

        def qk(qm, it, u, c):
            k0 = 0 if npg == 1 else off(it % npg, U * 128)
            kk = k_s.at[:, pl.ds(k0, U * 128)][c * kc // 2:(c + 1) * kc // 2, (u // HPS) * 128:(u // HPS + 1) * 128]
            kk = _unpack(kk)
            return _dot(kk, qm)

        def pv(it, u, c, s, m, l, o):
            rb = slab(it, u) * 64 + (u % HPS) * hr
            if not isinstance(rb, int):
                rb = pl.multiple_of(rb, hr)
            p = jnp.exp2(s - m)
            lc = _tree(jnp.add, p)
            oc = _dot(_unpack(vt_s[pl.ds(rb, hr), c * kc:(c + 1) * kc]), p.astype(bf16))
            return (lc if l is None else l + lc), (oc if o is None else o + oc)

        def finish(it, u, l, o):
            j = u % HPS
            ot_s[j * Dh:(j + 1) * Dh, :] = o * (1.0 / jnp.sum(l, axis=0, keepdims=True))
            if j == HPS - 1:
                o_s[pl.ds(off(it // npg, bq // 2), bq // 2), pl.ds(off(slab(it, u), 128), 128)] = _pack(ot_s[...].T)

        qm = masked_q(0, 0)
        mx = None
        for c in range(NC):
            s = qk(qm, 0, 0, c)
            sb[0][c * kc:(c + 1) * kc, :] = s
            mc = _tree(jnp.maximum, s)
            mx = mc if mx is None else jnp.maximum(mx, mc)
        sb[(UN - 1) % 4][(NC - lag) * kc:, :] = jnp.zeros((lag * kc, bq), f32)
        ot_s[...] = jnp.zeros_like(ot_s)
        st_mx[...] = mx
        st_m[...] = jnp.zeros_like(st_m)
        st_l[...] = jnp.ones_like(st_l)
        st_o[...] = jnp.zeros_like(st_o)
        for c in w_copies:
            c.wait()

        ko = D // go

        def wo_jobs(it):
            jobs = []
            for r in range(0, ko // n_it, 16):
                for n0 in range(0, ko, 128):
                    r0 = it * (ko // n_it) + r
                    load = lambda a, b, n0=n0, r0=r0: wo_v[pl.ds(pl.multiple_of(a * ko + r0, 16), 16), b * ko + n0:b * ko + n0 + 128]

                    def store(idx, v, n0=n0, r0=r0):
                        wo_c[pl.ds(pl.multiple_of(idx * (ko // 2) + r0 // 2, 8), 8), n0:n0 + 128] = v
                    jobs.extend((wo_v, n0, load, go, store, o) for o in (range(7) if lo > 1 else [None]))
            return jobs

        def p2(it, carry):
            it_prev = jnp.maximum(it - 1, 0)
            it_next = jnp.minimum(it + 1, n_it - 1)
            z = jnp.minimum(it, 0)
            m, l, o = st_m[...], st_l[...], st_o[...]
            mxs = {0: st_mx[...]}
            mx = qm = None
            jobs = wo_jobs(it)
            j0, j1 = 5 * NC, UN * NC - 8

            def ld(u, c):
                return sb[u % 4][pl.ds(pl.multiple_of(z + c * kc, kc), kc), :]

            for t in range(UN * NC):
                ua, ca = t // NC + 1, t % NC
                tb = t - lag
                ita, uu = (it, ua) if ua < UN else (it_next, 0)
                if ca == 0:
                    qm = masked_q(ita, uu)
                s = qk(qm, ita, uu, ca)
                sb[ua % 4][ca * kc:(ca + 1) * kc, :] = s
                mc = _tree(jnp.maximum, s)
                mx = mc if ca == 0 else jnp.maximum(mx, mc)
                if ca == NC - 1:
                    mxs[ua] = mx
                itb, ub, cb = (it_prev, UN - 1, NC + tb) if tb < 0 else (it, tb // NC, tb % NC)
                if cb == 0:
                    m = jnp.max(mxs[ub], axis=0, keepdims=True)
                    l = o = None
                l, o = pv(itb, ub, cb, ld(ub, cb), m, l, o)
                if cb == NC - 1:
                    finish(itb, ub, l, o)
                if j0 <= t < j1:
                    run_jobs(jobs, t - j0, j1 - j0, s, z)
            st_mx[...] = mxs[UN]
            st_m[...] = m
            st_l[...] = l
            st_o[...] = o
            return carry
        lax.fori_loop(0, n_it, p2, 0)
        m, l, o = st_m[...], st_l[...], st_o[...]
        for c in range(NC - lag, NC):
            l, o = pv(n_it - 1, UN - 1, c, sb[(UN - 1) % 4][c * kc:(c + 1) * kc, :], m, l, o)
        finish(n_it - 1, UN - 1, l, o)

        def o_copies(i, slot):
            hb = bm3 // 2
            return [pltpu.make_async_copy(out_v.at[slot, pl.ds(p * hb, hb)], out_hbm.at[pl.ds(i * bm3 + p * hb, hb)],
                                          sem_o.at[2 * slot + p]) for p in range(2)]

        def p3(i, carry):
            slot = i % 2

            @pl.when(i >= 2)
            def _():
                for c in o_copies(i - 2, slot):
                    c.wait()

            o = _unpack(o_s[pl.ds(pl.multiple_of(i * (bm3 // 2), bm3 // 2), bm3 // 2), :]).astype(f32)
            lops = [v.astype(bf16) for v in _lhs_ops(_grid(o, go))]
            att = _strassen(lambda j: _dot(lops[j], _unpack(wo_c[j * (ko // 2):(j + 1) * (ko // 2), :])), lo)
            to, hs = bm3 // go, []
            for a, row in enumerate(att):
                hs.append(x_v[pl.ds(pl.multiple_of(i * bm3 + a * to, to), to), :].astype(f32) + jnp.concatenate(row, axis=1))
            h = jnp.concatenate(hs, axis=0)
            y2 = _ln(h, keep_centered=False)
            ly = [v.astype(bf16) for v in _lhs_ops(_grid(y2, gm))]
            nin = 7 ** (lm - 1)
            b1 = b1_v[...].astype(f32).reshape(1, F)
            up = lambda j, f0: _dot(ly[j], _unpack(w1_c[j * (km // 2):(j + 1) * (km // 2), f0:f0 + fw]))
            early = {(j, f0): up(j, f0) for f0 in range(0, n_early * fw, fw)
                     for j in list(range(2 * nin, 3 * nin)) + list(range(4 * nin, 5 * nin))}
            tm = bm3 // gm
            for f0 in range(0, fm, fw):
                pre = _strassen(lambda j: early[j, f0] if (j, f0) in early else up(j, f0), lm)
                act = [[_gelu(blk + b1[:, gm * f0 + b * fw:gm * f0 + (b + 1) * fw]) for b, blk in enumerate(row)] for row in pre]
                for j, v in enumerate(_lhs_ops(act)):
                    g_s[j * (tm // 2):(j + 1) * (tm // 2), f0:f0 + fw] = _pack(v)
            down = _strassen(lambda j: _dot(_unpack(g_s[j * (tm // 2):(j + 1) * (tm // 2), :]),
                                            _unpack(w2_c[j * (fm // 2):(j + 1) * (fm // 2), :])), lm)
            res = _grid(h + b2_v[...].astype(f32).reshape(1, D), gm)
            for a, row in enumerate(down):
                for b, blk in enumerate(row):
                    out_v[slot, a * tm:(a + 1) * tm, b * km:(b + 1) * km] = (res[a][b] + blk).astype(bf16)
                if (a + 1) % (gm // 2) == 0:
                    o_copies(i, slot)[a // (gm // 2)].start()
            return carry
        lax.fori_loop(0, nb3, p3, 0)
        for c in o_copies(nb3 - 2, (nb3 - 2) % 2) + o_copies(nb3 - 1, (nb3 - 1) % 2):
            c.wait()

    any_spec = pl.BlockSpec(memory_space=pl.ANY)
    V = pltpu.VMEM
    return pl.pallas_call(
        kernel,
        out_shape=jax.ShapeDtypeStruct((S, D), bf16),
        in_specs=[any_spec] * 7,
        out_specs=any_spec,
        scratch_shapes=[
            V((S, D), bf16), *[V((D + PAD, WC), bf16)] * nwc, V((D + PAD, D), bf16),
            V((2 * D + PAD, gm * fw), bf16), V((F,), bf16), V((2 * gm * fw + PAD, D), bf16), V((D,), bf16),
            V((3 * 7 ** lq * D // gq // 2, D // gq), u32), V((7 ** lo * D // go // 2, D // go), u32),
            V((7 ** lm * D // gm // 2, F // gm), u32), V((7 ** lm * F // gm // 2, D // gm), u32),
            V((7 ** lq * bm1 // gq // 2, D // gq), u32), V((7 ** lm * bm3 // gm // 2, F // gm), u32),
            V((S // 2, D), u32), V((S // 2, D), u32), V((D // 2, S), u32), V((D // 2, S), u32),
            V((S, bq), f32), V((S, bq), f32), V((S, bq), f32), V((S, bq), f32), V((128, bq), f32),
            V((8, bq), f32), V((1, bq), f32), V((8, bq), f32), V((Dh, bq), f32),
            V((2, bm3, D), bf16),
            pltpu.SemaphoreType.DMA((nb1,)), pltpu.SemaphoreType.DMA((nwc,)),
            pltpu.SemaphoreType.DMA((3,)), pltpu.SemaphoreType.DMA((4,)), pltpu.SemaphoreType.DMA((4,)),
        ],
        compiler_params=pltpu.CompilerParams(vmem_limit_bytes=120 * 2**20),
        name="fused_block",
    )


@jax.jit
def pallas_sequential_preLN__softmax_full_mha__mixer_channel_mlp__prompt_kernel(
    A_x, A_wqkv, A_wo, B_x, B_w1, B_b1, B_w2, B_b2):
    del B_x
    B, S, D = A_x.shape
    F = B_w1.shape[1]
    out = make(S, D, F)(A_x.reshape(S, D), A_wqkv, A_wo, B_w1, B_b1, B_w2, B_b2)
    return out.reshape(B, S, D)
```

```python
import jax
import jax.numpy as jnp
from jax import lax
from jax.experimental import pallas as pl
from jax.experimental.pallas import tpu as pltpu

f32, bf16, u32 = jnp.float32, jnp.bfloat16, jnp.uint32

HEADS = 32
EPS = 1e-5
LOG2E = 1.4426950408889634

BM = 256
BQ = 256
KC = 128
LAG = 3
SLABS = 4
WC = 512
PAD = 16


def _tree(op, x):
    parts = [x[i * 8:(i + 1) * 8] for i in range(x.shape[0] // 8)]
    while len(parts) > 1:
        parts = [op(parts[i], parts[i + 1]) for i in range(0, len(parts), 2)]
    return parts[0]


def _ln(x, keep_centered=True):
    mu = jnp.mean(x, axis=-1, keepdims=True)
    xc = x - mu
    r = lax.rsqrt(jnp.mean(xc * xc, axis=-1, keepdims=True) + EPS)
    return xc * r if keep_centered else x * r - mu * r


def _gelu(x):
    c = 0.7978845608028654
    u = x * (c + (c * 0.044715) * (x * x))
    hx = 0.5 * x
    return hx + hx * jnp.tanh(u)


def _pack(x):
    return pltpu.bitcast(x.astype(bf16), u32)


def _unpack(x):
    return pltpu.bitcast(x, bf16)


def _dot(a, b):
    return jnp.dot(a, b, preferred_element_type=f32)


def _aligned(v, k):
    return v if isinstance(v, int) else pl.multiple_of(v, k)


def _grid(x, n):
    r, c = x.shape[0] // n, x.shape[1] // n
    return [[x[i * r:(i + 1) * r, j * c:(j + 1) * c] for j in range(n)] for i in range(n)]


def _add(a, b):
    return [[u + v for u, v in zip(ra, rb)] for ra, rb in zip(a, b)]


def _sub(a, b):
    return [[u - v for u, v in zip(ra, rb)] for ra, rb in zip(a, b)]


def _quads(g):
    h = len(g) // 2
    return [r[:h] for r in g[:h]], [r[h:] for r in g[:h]], [r[:h] for r in g[h:]], [r[h:] for r in g[h:]]


def _lhs_ops(g):
    if len(g) == 1:
        return [g[0][0]]
    a11, a12, a21, a22 = _quads(g)
    ops = (_add(a11, a22), _add(a21, a22), a11, a22, _add(a11, a12), _sub(a21, a11), _sub(a12, a22))
    return [v for q in ops for v in _lhs_ops(q)]


def _rhs_ops(g):
    if len(g) == 1:
        return [g[0][0]]
    b11, b12, b21, b22 = _quads(g)
    ops = (_add(b11, b22), b11, _sub(b12, b22), _sub(b21, b11), b22, _add(b11, b12), _add(b21, b22))
    return [v for q in ops for v in _rhs_ops(q)]


_RHS_TOP = ((_add, (0, 0), (1, 1)), (None, (0, 0), None), (_sub, (0, 1), (1, 1)), (_sub, (1, 0), (0, 0)),
            (None, (1, 1), None), (_add, (0, 0), (0, 1)), (_add, (1, 0), (1, 1)))


def _strassen(prod, level, base=0):
    if level == 0:
        return [[prod(base)]]
    m = lambda i: _strassen(prod, level - 1, base + i * 7 ** (level - 1))
    m3 = m(2)
    m5 = m(4)
    c12 = _add(m3, m5)
    m1 = m(0)
    c22 = _add(m1, m3)
    c11 = _sub(m1, m5)
    m4 = m(3)
    c11 = _add(_add(c11, m4), m(6))
    m2 = m(1)
    c21 = _add(m2, m4)
    c22 = _add(_sub(c22, m2), m(5))
    return [l + r for l, r in zip(c11, c12)] + [l + r for l, r in zip(c21, c22)]


def _make_call(S, D, F):
    Dh = D // HEADS
    HPS = 128 // Dh
    hr = Dh // 2
    nb = S // BM
    nwc = 3 * D // WC
    qscale = (Dh ** -0.5) * LOG2E
    tq, kq = BM // 2, D // 2
    tm, km, fm = BM // 4, D // 4, F // 4
    fw = fm // (nb - 1)
    pw = 4 * fw
    NC = S // KC
    UN = SLABS * HPS
    npg = D // 128 // SLABS
    n_it = (S // BQ) * npg
    assert WC == kq and fw % 128 == 0 and fw * (nb - 1) == fm and km == 16 * n_it and UN % 4 == 0

    def kernel(x_hbm, wqkv_hbm, wo_hbm, w1_hbm, b1_hbm, w2_hbm, b2_hbm, out_hbm,
               x_v, wq0, wq1, wq2, wq3, wq4, wq5, wo_v, w1_v, b1_v, w2_v, b2_v,
               wqkv_c, wo_c, w1_c, w2_c, l_s, g_s,
               o_s, k_s, qt_s, vt_s, sb0, sb1, sb2, sb3, ot_s, st_mx, st_m, st_l, st_o, out_v,
               sem_x, sem_q, sem_w, sem_p, sem_o):
        sb = [sb0, sb1, sb2, sb3]
        wq_v = [wq0, wq1, wq2, wq3, wq4, wq5]

        def x_copy(i):
            return pltpu.make_async_copy(x_hbm.at[pl.ds(i * BM, BM)], x_v.at[pl.ds(i * BM, BM)], sem_x.at[i])

        def q_copy(n):
            return pltpu.make_async_copy(wqkv_hbm.at[:, pl.ds(n * WC, WC)], wq_v[n].at[pl.ds(0, D)], sem_q.at[n])

        w_copies = [
            pltpu.make_async_copy(wo_hbm, wo_v.at[pl.ds(0, D)], sem_w.at[0]),
            pltpu.make_async_copy(b1_hbm, b1_v, sem_w.at[1]),
            pltpu.make_async_copy(b2_hbm, b2_v, sem_w.at[2]),
        ]

        def piece_copies(p, slot):
            f0 = _aligned(p * pw, pw)
            return [pltpu.make_async_copy(w1_hbm.at[:, pl.ds(f0, pw)], w1_v.at[pl.ds(slot * D, D)], sem_p.at[2 * slot]),
                    pltpu.make_async_copy(w2_hbm.at[pl.ds(f0, pw)], w2_v.at[pl.ds(slot * pw, pw)],
                                          sem_p.at[2 * slot + 1])]

        def fence(raw, col, val, z):
            top = raw.shape[0] - PAD
            row = pl.multiple_of(jnp.clip(z + top, 0, top), PAD)
            raw[pl.ds(row, PAD), col:col + 128] = val[0:PAD, 0:128].astype(bf16)

        def combine(load, store, top):
            quad = lambda a, b: [[load(2 * a + i, 2 * b + j).astype(f32) for j in range(2)] for i in range(2)]
            if top is None:
                ops, base = _rhs_ops(quad(0, 0)), 0
            else:
                op, a, b = _RHS_TOP[top]
                ops, base = _rhs_ops(quad(*a) if op is None else op(quad(*a), quad(*b))), 7 * top
            for idx, v in enumerate(ops):
                store(base + idx, _pack(v))

        def run_jobs(jobs, n, nslots, val, z):
            for raw, col, load, store, top in jobs[n * len(jobs) // nslots:(n + 1) * len(jobs) // nslots]:
                fence(raw, col, val, z)
                combine(load, store, top)

        def qkv_jobs(which):
            jobs = []
            for r0 in range(0, kq, 16):
                for n0 in range(0, kq, 128):
                    load = lambda a, b, r0=r0, n0=n0: wq_v[2 * which + b][a * kq + r0:a * kq + r0 + 16, n0:n0 + 128]

                    def store(idx, v, r0=r0, n0=n0):
                        r = (which * 7 + idx) * (kq // 2) + r0 // 2
                        wqkv_c[r:r + 8, n0:n0 + 128] = v
                    jobs.append((wq_v[2 * which], n0, load, store, None))
            return jobs

        def mlp_jobs(p, slot):
            jobs = []
            n1 = p * fw
            first_col = lambda t: 2 * _RHS_TOP[t][1][1]
            for r0 in range(0, km, 16):
                for c0 in range(0, fw, 128):
                    load = lambda a, b, r0=r0, c0=c0: w1_v[pl.ds(_aligned(slot * D + a * km + r0, 16), 16),
                                                           b * fw + c0:b * fw + c0 + 128]

                    def store(idx, v, r0=r0, c0=c0):
                        r = idx * (km // 2) + r0 // 2
                        w1_c[r:r + 8, pl.ds(_aligned(n1 + c0, 128), 128)] = v
                    jobs.extend((w1_v, first_col(t) * fw + c0, load, store, t) for t in range(7))
            for r0 in range(0, fw, 16):
                for c0 in range(0, km, 128):
                    load = lambda a, b, r0=r0, c0=c0: w2_v[pl.ds(_aligned((slot * 4 + a) * fw + r0, 16), 16),
                                                           b * km + c0:b * km + c0 + 128]

                    def store(idx, v, r0=r0, c0=c0):
                        w2_c[pl.ds(_aligned(idx * (fm // 2) + (n1 + r0) // 2, 8), 8), c0:c0 + 128] = v
                    jobs.extend((w2_v, first_col(t) * km + c0, load, store, t) for t in range(7))
            return jobs

        def wo_jobs(it):
            jobs = []
            r0 = it * 16
            for n0 in range(0, km, 128):
                load = lambda a, b, n0=n0: wo_v[pl.ds(pl.multiple_of(a * km + r0, 16), 16),
                                                b * km + n0:b * km + n0 + 128]

                def store(idx, v, n0=n0):
                    wo_c[pl.ds(pl.multiple_of(idx * (km // 2) + r0 // 2, 8), 8), n0:n0 + 128] = v
                jobs.extend((wo_v, n0, load, store, t) for t in range(7))
            return jobs

        def put_qkv(which, t0, c0, val):
            n, w = val.shape
            if which == 0:
                qt_s[c0 // 2:(c0 + w) // 2, pl.ds(t0, n)] = _pack((val * qscale).T)
            elif which == 2:
                vt_s[c0 // 2:(c0 + w) // 2, pl.ds(t0, n)] = _pack(val.T)
            else:
                k_s[pl.ds(_aligned(t0 // 2, n // 2), n // 2), c0:c0 + w] = _pack(val)

        def ln_operands(i):
            y = _ln(x_v[pl.ds(_aligned(i * BM, BM), BM), :].astype(f32))
            for j, v in enumerate(_lhs_ops(_grid(y, 2))):
                l_s[j * (tq // 2):(j + 1) * (tq // 2), :] = _pack(v)

        def opaque_zero():
            v = pltpu.bitcast(x_v[0:16, 0:128], jnp.int32)[0, 0]
            z = (v * v + v) & 1
            w = pltpu.bitcast(x_v[pl.ds(pl.multiple_of(z * 16, 16), 16), 0:128], jnp.int32)[0, 0]
            return v - w

        def plain(y, t0, chunks, jobs, z):
            nslots = len(chunks) * (WC // 128) * (y.shape[0] // 128) - 2
            n = 0
            for ch in chunks:
                for c in range(0, WC, 128):
                    w = wq_v[ch][0:D, c:c + 128]
                    for r in range(0, y.shape[0], 128):
                        v = _dot(y[r:r + 128], w)
                        put_qkv(ch * WC // D, t0 + r, (ch * WC + c) % D, v)
                        if n < nslots:
                            run_jobs(jobs, n, nslots, v, z)
                        n += 1

        x_copy(0).start()
        q_copy(0).start()
        x_copy(0).wait()
        x_copy(1).start()
        y0 = _ln(x_v[0:BM, :].astype(f32)).astype(bf16)
        z0 = opaque_zero()
        q_copy(0).wait()
        q_copy(1).start()
        q_copy(4).start()
        x_copy(1).wait()
        for cp in [q_copy(5)] + piece_copies(0, 0):
            cp.start()
        plain(y0, 0, [0], [], z0)
        y1 = _ln(x_v[BM:2 * BM, :].astype(f32)).astype(bf16)
        plain(y1, BM, [0], [], z0)
        y01 = jnp.concatenate([y0, y1], axis=0)
        q_copy(1).wait()
        q_copy(4).wait()
        for cp in (q_copy(2), q_copy(3), x_copy(2)):
            cp.start()
        plain(y01, 0, [1, 4], qkv_jobs(0), z0)
        for cp in [q_copy(5)] + piece_copies(0, 0):
            cp.wait()
        for cp in piece_copies(1, 1) + [x_copy(3)]:
            cp.start()
        jobs0 = mlp_jobs(0, 0)
        j1, j2 = len(jobs0) * 3 // 10, len(jobs0) * 9 // 10
        plain(y01, 0, [5], qkv_jobs(2) + jobs0[:j1], z0)
        q_copy(2).wait()
        q_copy(3).wait()
        x_copy(2).wait()
        plain(y01, 0, [2], jobs0[j1:j2], z0)
        plain(y01, 0, [3], jobs0[j2:] + qkv_jobs(1), z0)
        ln_operands(2)

        def qkv_block(i, carry):
            slot = (i - 1) % 2
            for cp in piece_copies(i - 1, slot):
                cp.wait()

            @pl.when(i + 1 < nb)
            def _():
                x_copy(i + 1).wait()
                for cp in piece_copies(i, 1 - slot):
                    cp.start()

            @pl.when(i + 2 < nb)
            def _():
                x_copy(i + 2).start()

            @pl.when(i == nb - 2)
            def _():
                for cp in w_copies:
                    cp.start()

            jobs = mlp_jobs(i - 1, slot)
            first, last = 8, 3 * 7 * (kq // 128) - 16
            count = [0]
            z = jnp.minimum(i, 0)

            for which in (0, 2, 1):
                def prod(j):
                    r = (which * 7 + j) * (kq // 2)
                    lhs = _unpack(l_s[j * (tq // 2):(j + 1) * (tq // 2), :])
                    cols = []
                    for c in range(0, kq, 128):
                        cols.append(_dot(lhs, _unpack(wqkv_c[r:r + kq // 2, c:c + 128])))
                        if first <= count[0] < last:
                            run_jobs(jobs, count[0] - first, last - first, cols[-1], z)
                        count[0] += 1
                    return jnp.concatenate(cols, axis=1)
                for a, row in enumerate(_strassen(prod, 1)):
                    for b, blk in enumerate(row):
                        put_qkv(which, pl.multiple_of(i * BM + a * tq, tq), b * kq, blk)
            ln_operands(jnp.minimum(i + 1, nb - 1))
            return carry
        lax.fori_loop(2, nb, qkv_block, 0)

        def masked_q(it, u):
            j = u % HPS
            r0 = _aligned(((it % npg) * SLABS + u // HPS) * 64 + j * hr, hr)
            parts = []
            if j > 0:
                parts.append(jnp.zeros((j * hr, BQ), u32))
            parts.append(qt_s[pl.ds(r0, hr), pl.ds(_aligned((it // npg) * BQ, BQ), BQ)])
            if j < HPS - 1:
                parts.append(jnp.zeros(((HPS - 1 - j) * hr, BQ), u32))
            return _unpack(jnp.concatenate(parts, axis=0))

        def scores(qm, it, u, c):
            k_view = k_s.at[:, pl.ds(_aligned((it % npg) * (SLABS * 128), SLABS * 128), SLABS * 128)]
            g = u // HPS
            return _dot(_unpack(k_view[c * KC // 2:(c + 1) * KC // 2, g * 128:(g + 1) * 128]), qm)

        def softmax_pv(it, u, c, s, m, l, o):
            r0 = _aligned(((it % npg) * SLABS + u // HPS) * 64 + (u % HPS) * hr, hr)
            p = jnp.exp2(s - m)
            lc = _tree(jnp.add, p)
            oc = _dot(_unpack(vt_s[pl.ds(r0, hr), c * KC:(c + 1) * KC]), p.astype(bf16))
            return (lc if l is None else l + lc), (oc if o is None else o + oc)

        def finish(it, u, l, o):
            j = u % HPS
            ot_s[j * Dh:(j + 1) * Dh, :] = o * (1.0 / jnp.sum(l, axis=0, keepdims=True))
            if j == HPS - 1:
                rows = pl.ds(_aligned((it // npg) * (BQ // 2), BQ // 2), BQ // 2)
                cols = pl.ds(_aligned(((it % npg) * SLABS + u // HPS) * 128, 128), 128)
                o_s[rows, cols] = _pack(ot_s[...].T)

        qm = masked_q(0, 0)
        mx = None
        for c in range(NC):
            s = scores(qm, 0, 0, c)
            sb[0][c * KC:(c + 1) * KC, :] = s
            mc = _tree(jnp.maximum, s)
            mx = mc if mx is None else jnp.maximum(mx, mc)
        sb[(UN - 1) % 4][(NC - LAG) * KC:, :] = jnp.zeros((LAG * KC, BQ), f32)
        ot_s[...] = jnp.zeros_like(ot_s)
        st_mx[...] = mx
        st_m[...] = jnp.zeros_like(st_m)
        st_l[...] = jnp.ones_like(st_l)
        st_o[...] = jnp.zeros_like(st_o)
        for cp in w_copies:
            cp.wait()

        def attention(it, carry):
            it_prev = jnp.maximum(it - 1, 0)
            it_next = jnp.minimum(it + 1, n_it - 1)
            z = jnp.minimum(it, 0)
            m, l, o = st_m[...], st_l[...], st_o[...]
            mxs = {0: st_mx[...]}
            mx = qm = None
            jobs = wo_jobs(it)
            first, last = 5 * NC, UN * NC - 8
            for t in range(UN * NC):
                ua, ca = t // NC + 1, t % NC
                ita, uu = (it, ua) if ua < UN else (it_next, 0)
                if ca == 0:
                    qm = masked_q(ita, uu)
                s = scores(qm, ita, uu, ca)
                sb[ua % 4][ca * KC:(ca + 1) * KC, :] = s
                mc = _tree(jnp.maximum, s)
                mx = mc if ca == 0 else jnp.maximum(mx, mc)
                if ca == NC - 1:
                    mxs[ua] = mx

                tb = t - LAG
                itb, ub, cb = (it_prev, UN - 1, NC + tb) if tb < 0 else (it, tb // NC, tb % NC)
                if cb == 0:
                    m = jnp.max(mxs[ub], axis=0, keepdims=True)
                    l = o = None
                sv = sb[ub % 4][pl.ds(pl.multiple_of(z + cb * KC, KC), KC), :]
                l, o = softmax_pv(itb, ub, cb, sv, m, l, o)
                if cb == NC - 1:
                    finish(itb, ub, l, o)
                if first <= t < last:
                    run_jobs(jobs, t - first, last - first, s, z)
            st_mx[...] = mxs[UN]
            st_m[...] = m
            st_l[...] = l
            st_o[...] = o
            return carry
        lax.fori_loop(0, n_it, attention, 0)
        m, l, o = st_m[...], st_l[...], st_o[...]
        for c in range(NC - LAG, NC):
            l, o = softmax_pv(n_it - 1, UN - 1, c, sb[(UN - 1) % 4][c * KC:(c + 1) * KC, :], m, l, o)
        finish(n_it - 1, UN - 1, l, o)

        def out_copy(i, slot, half):
            hb = BM // 2
            return pltpu.make_async_copy(out_v.at[slot, pl.ds(half * hb, hb)],
                                         out_hbm.at[pl.ds(i * BM + half * hb, hb)], sem_o.at[2 * slot + half])

        def mlp_block(i, carry):
            slot = i % 2

            @pl.when(i >= 2)
            def _():
                for half in range(2):
                    out_copy(i - 2, slot, half).wait()

            o = _unpack(o_s[pl.ds(pl.multiple_of(i * (BM // 2), BM // 2), BM // 2), :]).astype(f32)
            lo = [v.astype(bf16) for v in _lhs_ops(_grid(o, 4))]
            att = _strassen(lambda j: _dot(lo[j], _unpack(wo_c[j * (km // 2):(j + 1) * (km // 2), :])), 2)
            h = jnp.concatenate(
                [x_v[pl.ds(pl.multiple_of(i * BM + a * tm, tm), tm), :].astype(f32) + jnp.concatenate(row, axis=1)
                 for a, row in enumerate(att)], axis=0)
            ly = [v.astype(bf16) for v in _lhs_ops(_grid(_ln(h, keep_centered=False), 4))]
            b1 = b1_v[...].astype(f32).reshape(1, F)
            up = lambda j, f0: _dot(ly[j], _unpack(w1_c[j * (km // 2):(j + 1) * (km // 2), f0:f0 + fw]))
            early = {(j, f0): up(j, f0) for f0 in (0, fw) for j in list(range(14, 21)) + list(range(28, 35))}
            for f0 in range(0, fm, fw):
                pre = _strassen(lambda j: early[j, f0] if (j, f0) in early else up(j, f0), 2)
                act = [[_gelu(blk + b1[:, 4 * f0 + b * fw:4 * f0 + (b + 1) * fw]) for b, blk in enumerate(row)]
                       for row in pre]
                for j, v in enumerate(_lhs_ops(act)):
                    g_s[j * (tm // 2):(j + 1) * (tm // 2), f0:f0 + fw] = _pack(v)
            down = _strassen(lambda j: _dot(_unpack(g_s[j * (tm // 2):(j + 1) * (tm // 2), :]),
                                            _unpack(w2_c[j * (fm // 2):(j + 1) * (fm // 2), :])), 2)
            res = _grid(h + b2_v[...].astype(f32).reshape(1, D), 4)
            for a, row in enumerate(down):
                for b, blk in enumerate(row):
                    out_v[slot, a * tm:(a + 1) * tm, b * km:(b + 1) * km] = (res[a][b] + blk).astype(bf16)
                if a % 2 == 1:
                    out_copy(i, slot, a // 2).start()
            return carry
        lax.fori_loop(0, nb, mlp_block, 0)
        for i in (nb - 2, nb - 1):
            for half in range(2):
                out_copy(i, i % 2, half).wait()

    any_spec = pl.BlockSpec(memory_space=pl.ANY)
    V = pltpu.VMEM
    return pl.pallas_call(
        kernel,
        out_shape=jax.ShapeDtypeStruct((S, D), bf16),
        in_specs=[any_spec] * 7,
        out_specs=any_spec,
        scratch_shapes=[
            V((S, D), bf16), *[V((D + PAD, WC), bf16)] * nwc, V((D + PAD, D), bf16),
            V((2 * D + PAD, pw), bf16), V((F,), bf16), V((2 * pw + PAD, D), bf16), V((D,), bf16),
            V((3 * 7 * kq // 2, kq), u32), V((49 * km // 2, km), u32),
            V((49 * km // 2, fm), u32), V((49 * fm // 2, km), u32),
            V((7 * tq // 2, kq), u32), V((49 * tm // 2, fm), u32),
            V((S // 2, D), u32), V((S // 2, D), u32), V((D // 2, S), u32), V((D // 2, S), u32),
            V((S, BQ), f32), V((S, BQ), f32), V((S, BQ), f32), V((S, BQ), f32), V((128, BQ), f32),
            V((8, BQ), f32), V((1, BQ), f32), V((8, BQ), f32), V((Dh, BQ), f32),
            V((2, BM, D), bf16),
            pltpu.SemaphoreType.DMA((nb,)), pltpu.SemaphoreType.DMA((nwc,)), pltpu.SemaphoreType.DMA((3,)),
            pltpu.SemaphoreType.DMA((4,)), pltpu.SemaphoreType.DMA((4,)),
        ],
        compiler_params=pltpu.CompilerParams(vmem_limit_bytes=120 * 2 ** 20),
        name="fused_block",
    )


@jax.jit
def pallas_sequential_preLN__softmax_full_mha__mixer_channel_mlp__prompt_kernel(
    A_x: jax.Array,
    A_wqkv: jax.Array,
    A_wo: jax.Array,
    B_x: jax.Array,
    B_w1: jax.Array,
    B_b1: jax.Array,
    B_w2: jax.Array,
    B_b2: jax.Array,
):
    del B_x
    B, S, D = A_x.shape
    assert B == 1
    out = _make_call(S, D, B_w1.shape[1])(A_x.reshape(S, D), A_wqkv, A_wo, B_w1, B_b1, B_w2, B_b2)
    return out.reshape(B, S, D)
```

```python
import jax
import jax.numpy as jnp
from jax import lax
from jax.experimental import pallas as pl
from jax.experimental.pallas import tpu as pltpu

f32, bf16, u32 = jnp.float32, jnp.bfloat16, jnp.uint32

HEADS = 32
EPS = 1e-5
LOG2E = 1.4426950408889634

BM = 256
BQ = 256
KC = 128
LAG = 4
SLABS = 4
WC = 512
PAD = 16


def _tree(op, x):
    parts = [x[i * 8:(i + 1) * 8] for i in range(x.shape[0] // 8)]
    while len(parts) > 1:
        parts = [op(parts[i], parts[i + 1]) for i in range(0, len(parts), 2)]
    return parts[0]


def _ln(x, keep_centered=True):
    mu = jnp.mean(x, axis=-1, keepdims=True)
    xc = x - mu
    r = lax.rsqrt(jnp.mean(xc * xc, axis=-1, keepdims=True) + EPS)
    return xc * r if keep_centered else x * r - mu * r


def _gelu(x):
    c = 0.7978845608028654
    u = x * (c + (c * 0.044715) * (x * x))
    hx = 0.5 * x
    return hx + hx * jnp.tanh(u)


def _pack(x):
    return pltpu.bitcast(x.astype(bf16), u32)


def _unpack(x):
    return pltpu.bitcast(x, bf16)


def _dot(a, b):
    return jnp.dot(a, b, preferred_element_type=f32)


def _aligned(v, k):
    return v if isinstance(v, int) else pl.multiple_of(v, k)


def _grid(x, n):
    r, c = x.shape[0] // n, x.shape[1] // n
    return [[x[i * r:(i + 1) * r, j * c:(j + 1) * c] for j in range(n)] for i in range(n)]


def _add(a, b):
    return [[u + v for u, v in zip(ra, rb)] for ra, rb in zip(a, b)]


def _sub(a, b):
    return [[u - v for u, v in zip(ra, rb)] for ra, rb in zip(a, b)]


def _quads(g):
    h = len(g) // 2
    return [r[:h] for r in g[:h]], [r[h:] for r in g[:h]], [r[:h] for r in g[h:]], [r[h:] for r in g[h:]]


def _lhs_ops(g):
    if len(g) == 1:
        return [g[0][0]]
    a11, a12, a21, a22 = _quads(g)
    ops = (_add(a11, a22), _add(a21, a22), a11, a22, _add(a11, a12), _sub(a21, a11), _sub(a12, a22))
    return [v for q in ops for v in _lhs_ops(q)]


def _rhs_ops(g):
    if len(g) == 1:
        return [g[0][0]]
    b11, b12, b21, b22 = _quads(g)
    ops = (_add(b11, b22), b11, _sub(b12, b22), _sub(b21, b11), b22, _add(b11, b12), _add(b21, b22))
    return [v for q in ops for v in _rhs_ops(q)]


_RHS_TOP = ((_add, (0, 0), (1, 1)), (None, (0, 0), None), (_sub, (0, 1), (1, 1)), (_sub, (1, 0), (0, 0)),
            (None, (1, 1), None), (_add, (0, 0), (0, 1)), (_add, (1, 0), (1, 1)))


def _strassen(prod, level, base=0):
    if level == 0:
        return [[prod(base)]]
    m = lambda i: _strassen(prod, level - 1, base + i * 7 ** (level - 1))
    m3 = m(2)
    m5 = m(4)
    c12 = _add(m3, m5)
    m1 = m(0)
    c22 = _add(m1, m3)
    c11 = _sub(m1, m5)
    m4 = m(3)
    c11 = _add(_add(c11, m4), m(6))
    m2 = m(1)
    c21 = _add(m2, m4)
    c22 = _add(_sub(c22, m2), m(5))
    return [l + r for l, r in zip(c11, c12)] + [l + r for l, r in zip(c21, c22)]


def _make_call(S, D, F):
    Dh = D // HEADS
    HPS = 128 // Dh
    hr = Dh // 2
    nb = S // BM
    nwc = 3 * D // WC
    qscale = (Dh ** -0.5) * LOG2E
    tq, kq = BM // 2, D // 2
    tm, km, fm = BM // 4, D // 4, F // 4
    fw = fm // (nb - 1)
    pw = 4 * fw
    NC = S // KC
    UN = SLABS * HPS
    npg = D // 128 // SLABS
    n_it = (S // BQ) * npg
    assert WC == kq and fw % 128 == 0 and fw * (nb - 1) == fm and km % (16 * n_it) == 0 and UN % 4 == 0

    def kernel(x_hbm, wqkv_hbm, wo_hbm, w1_hbm, b1_hbm, w2_hbm, b2_hbm, out_hbm,
               x_v, wq0, wq1, wq2, wq3, wq4, wq5, wo_v, w1_v, b1_v, w2_v, b2_v,
               wqkv_c, wo_c, w1_c, w2_c, l_s, g_s,
               o_s, k_s, qt_s, vt_s, sb0, sb1, sb2, sb3, ot_s, st_mx, st_m, st_l, st_o, out_v,
               sem_x, sem_q, sem_w, sem_p, sem_o):
        sb = [sb0, sb1, sb2, sb3]
        wq_v = [wq0, wq1, wq2, wq3, wq4, wq5]

        def x_copy(i):
            return pltpu.make_async_copy(x_hbm.at[pl.ds(i * BM, BM)], x_v.at[pl.ds(i * BM, BM)], sem_x.at[i])

        def q_copy(n):
            return pltpu.make_async_copy(wqkv_hbm.at[:, pl.ds(n * WC, WC)], wq_v[n].at[pl.ds(0, D)], sem_q.at[n])

        w_copies = [
            pltpu.make_async_copy(wo_hbm, wo_v.at[pl.ds(0, D)], sem_w.at[0]),
            pltpu.make_async_copy(b1_hbm, b1_v, sem_w.at[1]),
            pltpu.make_async_copy(b2_hbm, b2_v, sem_w.at[2]),
        ]

        def piece_copies(p, slot):
            f0 = _aligned(p * pw, pw)
            return [pltpu.make_async_copy(w1_hbm.at[:, pl.ds(f0, pw)], w1_v.at[pl.ds(slot * D, D)], sem_p.at[2 * slot]),
                    pltpu.make_async_copy(w2_hbm.at[pl.ds(f0, pw)], w2_v.at[pl.ds(slot * pw, pw)],
                                          sem_p.at[2 * slot + 1])]

        def fence(raw, col, val, z):
            top = raw.shape[0] - PAD
            row = pl.multiple_of(jnp.clip(z + top, 0, top), PAD)
            raw[pl.ds(row, PAD), col:col + 128] = val[0:PAD, 0:128].astype(bf16)

        def combine(load, store, top):
            quad = lambda a, b: [[load(2 * a + i, 2 * b + j).astype(f32) for j in range(2)] for i in range(2)]
            if top is None:
                ops, base = _rhs_ops(quad(0, 0)), 0
            else:
                op, a, b = _RHS_TOP[top]
                ops, base = _rhs_ops(quad(*a) if op is None else op(quad(*a), quad(*b))), 7 * top
            for idx, v in enumerate(ops):
                store(base + idx, _pack(v))

        def run_jobs(jobs, n, nslots, val, z):
            for raw, col, load, store, top in jobs[n * len(jobs) // nslots:(n + 1) * len(jobs) // nslots]:
                fence(raw, col, val, z)
                combine(load, store, top)

        def qkv_jobs(which):
            jobs = []
            for r0 in range(0, kq, 16):
                for n0 in range(0, kq, 128):
                    load = lambda a, b, r0=r0, n0=n0: wq_v[2 * which + b][a * kq + r0:a * kq + r0 + 16, n0:n0 + 128]

                    def store(idx, v, r0=r0, n0=n0):
                        r = (which * 7 + idx) * (kq // 2) + r0 // 2
                        wqkv_c[r:r + 8, n0:n0 + 128] = v
                    jobs.append((wq_v[2 * which], n0, load, store, None))
            return jobs

        def mlp_jobs(p, slot):
            jobs = []
            n1 = p * fw
            first_col = lambda t: 2 * _RHS_TOP[t][1][1]
            for r0 in range(0, km, 16):
                for c0 in range(0, fw, 128):
                    load = lambda a, b, r0=r0, c0=c0: w1_v[pl.ds(_aligned(slot * D + a * km + r0, 16), 16),
                                                           b * fw + c0:b * fw + c0 + 128]

                    def store(idx, v, r0=r0, c0=c0):
                        r = idx * (km // 2) + r0 // 2
                        w1_c[r:r + 8, pl.ds(_aligned(n1 + c0, 128), 128)] = v
                    jobs.extend((w1_v, first_col(t) * fw + c0, load, store, t) for t in range(7))
            for r0 in range(0, fw, 16):
                for c0 in range(0, km, 128):
                    load = lambda a, b, r0=r0, c0=c0: w2_v[pl.ds(_aligned((slot * 4 + a) * fw + r0, 16), 16),
                                                           b * km + c0:b * km + c0 + 128]

                    def store(idx, v, r0=r0, c0=c0):
                        w2_c[pl.ds(_aligned(idx * (fm // 2) + (n1 + r0) // 2, 8), 8), c0:c0 + 128] = v
                    jobs.extend((w2_v, first_col(t) * km + c0, load, store, t) for t in range(7))
            return jobs

        def wo_jobs(it):
            jobs = []
            for r in range(0, km // n_it, 16):
                r0 = it * (km // n_it) + r
                for n0 in range(0, km, 128):
                    load = lambda a, b, r0=r0, n0=n0: wo_v[pl.ds(pl.multiple_of(a * km + r0, 16), 16),
                                                           b * km + n0:b * km + n0 + 128]

                    def store(idx, v, r0=r0, n0=n0):
                        wo_c[pl.ds(pl.multiple_of(idx * (km // 2) + r0 // 2, 8), 8), n0:n0 + 128] = v
                    jobs.extend((wo_v, n0, load, store, t) for t in range(7))
            return jobs

        def put_qkv(which, t0, c0, val):
            n, w = val.shape
            if which == 0:
                qt_s[c0 // 2:(c0 + w) // 2, pl.ds(t0, n)] = _pack((val * qscale).T)
            elif which == 2:
                vt_s[c0 // 2:(c0 + w) // 2, pl.ds(t0, n)] = _pack(val.T)
            else:
                k_s[pl.ds(_aligned(t0 // 2, n // 2), n // 2), c0:c0 + w] = _pack(val)

        def ln_operands(i):
            y = _ln(x_v[pl.ds(_aligned(i * BM, BM), BM), :].astype(f32))
            for j, v in enumerate(_lhs_ops(_grid(y, 2))):
                l_s[j * (tq // 2):(j + 1) * (tq // 2), :] = _pack(v)

        def opaque_zero():
            v = pltpu.bitcast(x_v[0:16, 0:128], jnp.int32)[0, 0]
            z = (v * v + v) & 1
            w = pltpu.bitcast(x_v[pl.ds(pl.multiple_of(z * 16, 16), 16), 0:128], jnp.int32)[0, 0]
            return v - w

        def plain(y, t0, chunks, jobs, z):
            nslots = len(chunks) * (WC // 128) * (y.shape[0] // 128) - 2
            n = 0
            for ch in chunks:
                for c in range(0, WC, 128):
                    w = wq_v[ch][0:D, c:c + 128]
                    for r in range(0, y.shape[0], 128):
                        v = _dot(y[r:r + 128], w)
                        put_qkv(ch * WC // D, t0 + r, (ch * WC + c) % D, v)
                        if n < nslots:
                            run_jobs(jobs, n, nslots, v, z)
                        n += 1

        x_copy(0).start()
        q_copy(0).start()
        x_copy(0).wait()
        x_copy(1).start()
        y0 = _ln(x_v[0:BM, :].astype(f32)).astype(bf16)
        z0 = opaque_zero()
        q_copy(0).wait()
        q_copy(1).start()
        q_copy(4).start()
        x_copy(1).wait()
        for cp in [q_copy(5)] + piece_copies(0, 0):
            cp.start()
        plain(y0, 0, [0], [], z0)
        y1 = _ln(x_v[BM:2 * BM, :].astype(f32)).astype(bf16)
        plain(y1, BM, [0], [], z0)
        y01 = jnp.concatenate([y0, y1], axis=0)
        q_copy(1).wait()
        q_copy(4).wait()
        for cp in (q_copy(2), q_copy(3), x_copy(2)):
            cp.start()
        plain(y01, 0, [1, 4], qkv_jobs(0), z0)
        for cp in [q_copy(5)] + piece_copies(0, 0):
            cp.wait()
        for cp in piece_copies(1, 1) + [x_copy(3)]:
            cp.start()
        jobs0 = mlp_jobs(0, 0)
        j1, j2 = len(jobs0) * 3 // 10, len(jobs0) * 9 // 10
        plain(y01, 0, [5], qkv_jobs(2) + jobs0[:j1], z0)
        q_copy(2).wait()
        q_copy(3).wait()
        x_copy(2).wait()
        plain(y01, 0, [2], jobs0[j1:j2], z0)
        plain(y01, 0, [3], jobs0[j2:] + qkv_jobs(1), z0)
        ln_operands(2)

        def qkv_block(i, carry):
            slot = (i - 1) % 2
            for cp in piece_copies(i - 1, slot):
                cp.wait()

            @pl.when(i + 1 < nb)
            def _():
                x_copy(i + 1).wait()
                for cp in piece_copies(i, 1 - slot):
                    cp.start()

            @pl.when(i + 2 < nb)
            def _():
                x_copy(i + 2).start()

            @pl.when(i == nb - 2)
            def _():
                for cp in w_copies:
                    cp.start()

            jobs = mlp_jobs(i - 1, slot)
            first, last = 9, 3 * 7 * (kq // 128) - 17
            count = [0]
            z = jnp.minimum(i, 0)

            for which in (0, 2, 1):
                def prod(j):
                    r = (which * 7 + j) * (kq // 2)
                    lhs = _unpack(l_s[j * (tq // 2):(j + 1) * (tq // 2), :])
                    cols = []
                    for c in range(0, kq, 128):
                        cols.append(_dot(lhs, _unpack(wqkv_c[r:r + kq // 2, c:c + 128])))
                        if first <= count[0] < last:
                            run_jobs(jobs, count[0] - first, last - first, cols[-1], z)
                        count[0] += 1
                    return jnp.concatenate(cols, axis=1)
                for a, row in enumerate(_strassen(prod, 1)):
                    for b, blk in enumerate(row):
                        put_qkv(which, pl.multiple_of(i * BM + a * tq, tq), b * kq, blk)
            ln_operands(jnp.minimum(i + 1, nb - 1))
            return carry
        lax.fori_loop(2, nb, qkv_block, 0)

        def masked_q(it, u):
            j = u % HPS
            r0 = _aligned(((it % npg) * SLABS + u // HPS) * 64 + j * hr, hr)
            parts = []
            if j > 0:
                parts.append(jnp.zeros((j * hr, BQ), u32))
            parts.append(qt_s[pl.ds(r0, hr), pl.ds(_aligned((it // npg) * BQ, BQ), BQ)])
            if j < HPS - 1:
                parts.append(jnp.zeros(((HPS - 1 - j) * hr, BQ), u32))
            return _unpack(jnp.concatenate(parts, axis=0))

        def scores(qm, it, u, c):
            k_view = k_s.at[:, pl.ds(_aligned((it % npg) * (SLABS * 128), SLABS * 128), SLABS * 128)]
            g = u // HPS
            return _dot(_unpack(k_view[c * KC // 2:(c + 1) * KC // 2, g * 128:(g + 1) * 128]), qm)

        def softmax_pv(it, u, c, s, m, l, o):
            r0 = _aligned(((it % npg) * SLABS + u // HPS) * 64 + (u % HPS) * hr, hr)
            p = jnp.exp2(s - m)
            lc = _tree(jnp.add, p)
            oc = _dot(_unpack(vt_s[pl.ds(r0, hr), c * KC:(c + 1) * KC]), p.astype(bf16))
            return (lc if l is None else l + lc), (oc if o is None else o + oc)

        def finish(it, u, l, o):
            j = u % HPS
            ot_s[j * Dh:(j + 1) * Dh, :] = o * (1.0 / jnp.sum(l, axis=0, keepdims=True))
            if j == HPS - 1:
                rows = pl.ds(_aligned((it // npg) * (BQ // 2), BQ // 2), BQ // 2)
                cols = pl.ds(_aligned(((it % npg) * SLABS + u // HPS) * 128, 128), 128)
                o_s[rows, cols] = _pack(ot_s[...].T)

        qm = masked_q(0, 0)
        mx = None
        for c in range(NC):
            s = scores(qm, 0, 0, c)
            sb[0][c * KC:(c + 1) * KC, :] = s
            mc = _tree(jnp.maximum, s)
            mx = mc if mx is None else jnp.maximum(mx, mc)
        sb[(UN - 1) % 4][(NC - LAG) * KC:, :] = jnp.zeros((LAG * KC, BQ), f32)
        ot_s[...] = jnp.zeros_like(ot_s)
        st_mx[...] = mx
        st_m[...] = jnp.zeros_like(st_m)
        st_l[...] = jnp.ones_like(st_l)
        st_o[...] = jnp.zeros_like(st_o)
        for cp in w_copies:
            cp.wait()

        def attention(it, carry):
            it_prev = jnp.maximum(it - 1, 0)
            it_next = jnp.minimum(it + 1, n_it - 1)
            z = jnp.minimum(it, 0)
            m, l, o = st_m[...], st_l[...], st_o[...]
            mxs = {0: st_mx[...]}
            mx = qm = None
            jobs = wo_jobs(it)
            first, last = 10 * NC, UN * NC - NC
            for t in range(UN * NC):
                ua, ca = t // NC + 1, t % NC
                ita, uu = (it, ua) if ua < UN else (it_next, 0)
                if ca == 0:
                    qm = masked_q(ita, uu)
                s = scores(qm, ita, uu, ca)
                sb[ua % 4][ca * KC:(ca + 1) * KC, :] = s
                mc = _tree(jnp.maximum, s)
                mx = mc if ca == 0 else jnp.maximum(mx, mc)
                if ca == NC - 1:
                    mxs[ua] = mx

                tb = t - LAG
                itb, ub, cb = (it_prev, UN - 1, NC + tb) if tb < 0 else (it, tb // NC, tb % NC)
                if cb == 0:
                    m = jnp.max(mxs[ub], axis=0, keepdims=True)
                    l = o = None
                sv = sb[ub % 4][pl.ds(pl.multiple_of(z + cb * KC, KC), KC), :]
                l, o = softmax_pv(itb, ub, cb, sv, m, l, o)
                if cb == NC - 1:
                    finish(itb, ub, l, o)
                if first <= t < last:
                    run_jobs(jobs, t - first, last - first, s, z)
            st_mx[...] = mxs[UN]
            st_m[...] = m
            st_l[...] = l
            st_o[...] = o
            return carry
        lax.fori_loop(0, n_it, attention, 0)
        m, l, o = st_m[...], st_l[...], st_o[...]
        for c in range(NC - LAG, NC):
            l, o = softmax_pv(n_it - 1, UN - 1, c, sb[(UN - 1) % 4][c * KC:(c + 1) * KC, :], m, l, o)
        finish(n_it - 1, UN - 1, l, o)

        def out_copy(i, slot, half):
            hb = BM // 2
            return pltpu.make_async_copy(out_v.at[slot, pl.ds(half * hb, hb)],
                                         out_hbm.at[pl.ds(i * BM + half * hb, hb)], sem_o.at[2 * slot + half])

        def mlp_block(i, carry):
            slot = i % 2

            @pl.when(i >= 2)
            def _():
                for half in range(2):
                    out_copy(i - 2, slot, half).wait()

            o = _unpack(o_s[pl.ds(pl.multiple_of(i * (BM // 2), BM // 2), BM // 2), :]).astype(f32)
            lo = [v.astype(bf16) for v in _lhs_ops(_grid(o, 4))]
            att = _strassen(lambda j: _dot(lo[j], _unpack(wo_c[j * (km // 2):(j + 1) * (km // 2), :])), 2)
            h = jnp.concatenate(
                [x_v[pl.ds(pl.multiple_of(i * BM + a * tm, tm), tm), :].astype(f32) + jnp.concatenate(row, axis=1)
                 for a, row in enumerate(att)], axis=0)
            ly = [v.astype(bf16) for v in _lhs_ops(_grid(_ln(h, keep_centered=False), 4))]
            b1 = b1_v[...].astype(f32).reshape(1, F)
            up = lambda j, f0: _dot(ly[j], _unpack(w1_c[j * (km // 2):(j + 1) * (km // 2), f0:f0 + fw]))
            early = {(j, f0): up(j, f0) for f0 in (0, fw) for j in list(range(14, 21)) + list(range(28, 35))}
            for f0 in range(0, fm, fw):
                pre = _strassen(lambda j: early[j, f0] if (j, f0) in early else up(j, f0), 2)
                act = [[_gelu(blk + b1[:, 4 * f0 + b * fw:4 * f0 + (b + 1) * fw]) for b, blk in enumerate(row)]
                       for row in pre]
                for j, v in enumerate(_lhs_ops(act)):
                    g_s[j * (tm // 2):(j + 1) * (tm // 2), f0:f0 + fw] = _pack(v)
            down = _strassen(lambda j: _dot(_unpack(g_s[j * (tm // 2):(j + 1) * (tm // 2), :]),
                                            _unpack(w2_c[j * (fm // 2):(j + 1) * (fm // 2), :])), 2)
            res = _grid(h + b2_v[...].astype(f32).reshape(1, D), 4)
            for a, row in enumerate(down):
                for b, blk in enumerate(row):
                    out_v[slot, a * tm:(a + 1) * tm, b * km:(b + 1) * km] = (res[a][b] + blk).astype(bf16)
                if a % 2 == 1:
                    out_copy(i, slot, a // 2).start()
            return carry
        lax.fori_loop(0, nb, mlp_block, 0)
        for i in (nb - 2, nb - 1):
            for half in range(2):
                out_copy(i, i % 2, half).wait()

    any_spec = pl.BlockSpec(memory_space=pl.ANY)
    V = pltpu.VMEM
    return pl.pallas_call(
        kernel,
        out_shape=jax.ShapeDtypeStruct((S, D), bf16),
        in_specs=[any_spec] * 7,
        out_specs=any_spec,
        scratch_shapes=[
            V((S, D), bf16), *[V((D + PAD, WC), bf16)] * nwc, V((D + PAD, D), bf16),
            V((2 * D + PAD, pw), bf16), V((F,), bf16), V((2 * pw + PAD, D), bf16), V((D,), bf16),
            V((3 * 7 * kq // 2, kq), u32), V((49 * km // 2, km), u32),
            V((49 * km // 2, fm), u32), V((49 * fm // 2, km), u32),
            V((7 * tq // 2, kq), u32), V((49 * tm // 2, fm), u32),
            V((S // 2, D), u32), V((S // 2, D), u32), V((D // 2, S), u32), V((D // 2, S), u32),
            V((S, BQ), f32), V((S, BQ), f32), V((S, BQ), f32), V((S, BQ), f32), V((128, BQ), f32),
            V((8, BQ), f32), V((1, BQ), f32), V((8, BQ), f32), V((Dh, BQ), f32),
            V((2, BM, D), bf16),
            pltpu.SemaphoreType.DMA((nb,)), pltpu.SemaphoreType.DMA((nwc,)), pltpu.SemaphoreType.DMA((3,)),
            pltpu.SemaphoreType.DMA((4,)), pltpu.SemaphoreType.DMA((4,)),
        ],
        compiler_params=pltpu.CompilerParams(vmem_limit_bytes=120 * 2 ** 20),
        name="fused_block",
    )


@jax.jit
def pallas_sequential_preLN__softmax_full_mha__mixer_channel_mlp__prompt_kernel(
    A_x: jax.Array,
    A_wqkv: jax.Array,
    A_wo: jax.Array,
    B_x: jax.Array,
    B_w1: jax.Array,
    B_b1: jax.Array,
    B_w2: jax.Array,
    B_b2: jax.Array,
):
    del B_x
    B, S, D = A_x.shape
    assert B == 1
    out = _make_call(S, D, B_w1.shape[1])(A_x.reshape(S, D), A_wqkv, A_wo, B_w1, B_b1, B_w2, B_b2)
    return out.reshape(B, S, D)
```
